```python
import os as _os
_os.environ.setdefault("JAX_PLATFORMS", "cpu")
import jax
import jax.numpy as jnp

def _softmax(x, axis=-1):
    return jax.nn.softmax(x, axis=axis)
def _gelu(x):
    return jax.nn.gelu(x, approximate=True)
def _silu(x):
    return jax.nn.silu(x)
def _sigmoid(x):
    return jax.nn.sigmoid(x)
def _layernorm(x, axis=-1, eps=1e-5):
    m = jnp.mean(x, axis=axis, keepdims=True)
    v = jnp.var(x, axis=axis, keepdims=True)
    return (x - m) / jnp.sqrt(v + eps)
def _scatter_add(tgt, idx, src, axis=0):
    return tgt.at[idx].add(src)
def _segment_sum(src, seg, n):
    return jax.ops.segment_sum(src, seg, n)
class _Rng:
    def __init__(self, key):
        self._k = key
    def _next(self):
        self._k, sub = jax.random.split(self._k)
        return sub
    def normal(self, shape):
        return jax.random.normal(self._next(), shape, dtype=jnp.bfloat16)
    def randint(self, lo, hi, shape):
        return jax.random.randint(self._next(), shape, lo, hi, dtype=jnp.int32)
    def uniform(self, shape, lo=0.0, hi=1.0):
        return jax.random.uniform(self._next(), shape, jnp.bfloat16, lo, hi)
    def permutation(self, n):
        return jax.random.permutation(self._next(), n)


kernel_name = 'standalone__instancenorm__sampling'

def setup_inputs():
    _rng = _Rng(jax.random.key(int.from_bytes(__import__("os").urandom(4), "little")))
    _w = (lambda a: (lambda t: t.astype(jnp.bfloat16) if jnp.issubdtype(t.dtype, jnp.floating) else t)(jnp.asarray(a)))
    B, C, H, W = 16, 640, 16, 32
    return {
        "x": _w((lambda *s: _rng.normal(s) * 0.05)(B, C, H, W)),
        "g": _w((lambda *s: _rng.normal(s) * 0.05)(C) + 1.0),
        "b": _w((lambda *s: _rng.normal(s) * 0.05)(C)),
    }

def reference(x, g, b):
    mu = x.mean(axis=(-2, -1), keepdims=True)
    var = ((x - mu) * (x - mu)).mean(axis=(-2, -1), keepdims=True)
    xhat = (x - mu) / jnp.sqrt(var + 1e-5)
    return xhat * g.reshape(1, -1, 1, 1) + b.reshape(1, -1, 1, 1)
```

```python
import jax
import jax.numpy as jnp
import jax.experimental.pallas as pl
import jax.experimental.pallas.tpu as pltpu

_EPS = 1e-5
_DEPTH = 4


@jax.jit
def pallas_standalone__instancenorm__sampling_kernel(
    x: jax.Array,
    g: jax.Array,
    b: jax.Array,
):
    B, C, H, W = x.shape
    HW = H * W
    depth = min(_DEPTH, B)
    xt = x.transpose(0, 2, 3, 1).reshape(B, HW, C)

    def kernel_function(x_hbm, g_hbm, b_hbm, o_hbm, buf, g_v, b_v, rsem, gsem, wsem):
        def rd(k):
            return pltpu.make_async_copy(x_hbm.at[k], buf.at[k], rsem.at[k % depth])

        gc = pltpu.make_async_copy(g_hbm, g_v, gsem.at[0])
        bc = pltpu.make_async_copy(b_hbm, b_v, gsem.at[1])
        gc.start()
        bc.start()
        for k in range(depth):
            rd(k).start()
        gc.wait()
        bc.wait()
        gf = g_v[...].astype(jnp.float32).reshape(1, C)
        bf = b_v[...].astype(jnp.float32).reshape(1, C)

        nfirst = B - 1
        w1 = pltpu.make_async_copy(
            buf.at[pl.ds(0, nfirst)], o_hbm.at[pl.ds(0, nfirst)], wsem.at[0])
        w2 = pltpu.make_async_copy(
            buf.at[pl.ds(nfirst, 1)], o_hbm.at[pl.ds(nfirst, 1)], wsem.at[1])

        for k in range(B):
            rd(k).wait()
            if k + depth < B:
                rd(k + depth).start()
            xf = buf[k].astype(jnp.float32)
            mu = jnp.mean(xf, axis=0, keepdims=True)
            xc = xf - mu
            var = jnp.mean(xc * xc, axis=0, keepdims=True)
            scale = jax.lax.rsqrt(var + _EPS) * gf
            buf[k] = (xc * scale + bf).astype(buf.dtype)
            if k == nfirst - 1:
                w1.start()
        w2.start()
        w1.wait()
        w2.wait()

    out = pl.pallas_call(
        kernel_function,
        in_specs=[pl.BlockSpec(memory_space=pl.ANY)] * 3,
        out_specs=pl.BlockSpec(memory_space=pl.ANY),
        out_shape=jax.ShapeDtypeStruct((B, HW, C), x.dtype),
        scratch_shapes=[
            pltpu.VMEM((B, HW, C), x.dtype),
            pltpu.VMEM((C,), g.dtype),
            pltpu.VMEM((C,), b.dtype),
            pltpu.SemaphoreType.DMA((depth,)),
            pltpu.SemaphoreType.DMA((2,)),
            pltpu.SemaphoreType.DMA((2,)),
        ],
        compiler_params=pltpu.CompilerParams(vmem_limit_bytes=64 * 1024 * 1024),
    )(xt, g, b)
    return out.reshape(B, H, W, C).transpose(0, 3, 1, 2)
```

```python
import jax
import jax.numpy as jnp
import jax.experimental.pallas as pl
import jax.experimental.pallas.tpu as pltpu

_EPS = 1e-5
_DEPTH = 3
_GROUPS = 8
_PIECE_ROWS = 16


@jax.jit
def pallas_standalone__instancenorm__sampling_kernel(
    x: jax.Array,
    g: jax.Array,
    b: jax.Array,
):
    B, C, H, W = x.shape
    HW = H * W
    G = _GROUPS if B % _GROUPS == 0 else 1
    NB = B // G
    P = _PIECE_ROWS if HW % _PIECE_ROWS == 0 else HW
    depth = min(_DEPTH, B)

    xt = x.transpose(0, 2, 3, 1).reshape(G, NB, HW, C)

    def kernel_function(x_hbm, g_hbm, b_hbm, o_hbm, buf, g_v, b_v, rsem, sem):
        def read(k):
            gi, i = divmod(k, NB)
            return pltpu.make_async_copy(
                x_hbm.at[gi, i], buf.at[gi, i], rsem.at[k % depth])

        def start_writes(i):
            for j in range(HW // P):
                rows = pl.ds(j * P, P)
                pltpu.make_async_copy(
                    buf.at[:, i, rows], o_hbm.at[:, i, rows], sem).start()

        g_copy = pltpu.make_async_copy(g_hbm, g_v, sem)
        b_copy = pltpu.make_async_copy(b_hbm, b_v, sem)
        g_copy.start()
        b_copy.start()
        for k in range(depth):
            read(k).start()
        g_copy.wait()
        b_copy.wait()
        gf = g_v[...].astype(jnp.float32).reshape(1, C)
        bf = b_v[...].astype(jnp.float32).reshape(1, C)

        for k in range(B):
            read(k).wait()
            if k + depth < B:
                read(k + depth).start()
            gi, i = divmod(k, NB)
            xf = buf[gi, i].astype(jnp.float32)
            mu = jnp.mean(xf, axis=0, keepdims=True)
            xc = xf - mu
            var = jnp.mean(xc * xc, axis=0, keepdims=True)
            scale = jax.lax.rsqrt(var + _EPS) * gf
            buf[gi, i] = (xc * scale + bf).astype(buf.dtype)
            if k == B - 2:
                for i2 in range(NB - 1):
                    start_writes(i2)
        start_writes(NB - 1)
        pltpu.make_async_copy(buf, o_hbm, sem).wait()

    out = pl.pallas_call(
        kernel_function,
        in_specs=[pl.BlockSpec(memory_space=pl.ANY)] * 3,
        out_specs=pl.BlockSpec(memory_space=pl.ANY),
        out_shape=jax.ShapeDtypeStruct((G, NB, HW, C), x.dtype),
        scratch_shapes=[
            pltpu.VMEM((G, NB, HW, C), x.dtype),
            pltpu.VMEM((C,), g.dtype),
            pltpu.VMEM((C,), b.dtype),
            pltpu.SemaphoreType.DMA((depth,)),
            pltpu.SemaphoreType.DMA,
        ],
        compiler_params=pltpu.CompilerParams(vmem_limit_bytes=64 * 1024 * 1024),
    )(xt, g, b)
    return out.reshape(B, H, W, C).transpose(0, 3, 1, 2)
```
